```python
import os as _os
_os.environ.setdefault("JAX_PLATFORMS", "cpu")
import jax
import jax.numpy as jnp

def _softmax(x, axis=-1):
    return jax.nn.softmax(x, axis=axis)
def _gelu(x):
    return jax.nn.gelu(x, approximate=True)
def _silu(x):
    return jax.nn.silu(x)
def _sigmoid(x):
    return jax.nn.sigmoid(x)
def _layernorm(x, axis=-1, eps=1e-5):
    m = jnp.mean(x, axis=axis, keepdims=True)
    v = jnp.var(x, axis=axis, keepdims=True)
    return (x - m) / jnp.sqrt(v + eps)
def _scatter_add(tgt, idx, src, axis=0):
    return tgt.at[idx].add(src)
def _segment_sum(src, seg, n):
    return jax.ops.segment_sum(src, seg, n)
class _Rng:
    def __init__(self, key):
        self._k = key
    def _next(self):
        self._k, sub = jax.random.split(self._k)
        return sub
    def normal(self, shape):
        return jax.random.normal(self._next(), shape, dtype=jnp.bfloat16)
    def randint(self, lo, hi, shape):
        return jax.random.randint(self._next(), shape, lo, hi, dtype=jnp.int32)
    def uniform(self, shape, lo=0.0, hi=1.0):
        return jax.random.uniform(self._next(), shape, jnp.bfloat16, lo, hi)
    def permutation(self, n):
        return jax.random.permutation(self._next(), n)


kernel_name = 'sequential_preLN__linear_kernel_hedgehog__dense_activation_squared_relu__prompt'

def setup_inputs():
    _rng = _Rng(jax.random.key(int.from_bytes(__import__("os").urandom(4), "little")))
    _w = (lambda a: (lambda t: t.astype(jnp.bfloat16) if jnp.issubdtype(t.dtype, jnp.floating) else t)(jnp.asarray(a)))
    def _A_setup():
        B, S, D, H = 1, 2048, 512, 32
        Dh = D // H
        return {
            "x": _w((lambda *s: _rng.normal(s) * 0.05)(B, S, D)),
            "wqkv": _w((lambda *s: _rng.normal(s) * 0.2)(D, 3 * D)),
            "w_phi": _w((lambda *s: _rng.normal(s) * 0.2)(H, Dh, Dh) * (Dh ** -0.5)),
            "wo": _w((lambda *s: _rng.normal(s) * 0.05)(D, D)),
        }
    _A_in = _A_setup()

    def _B_setup():
        B, S, D, F = 1, 2048, 512, 1792
        return {
            "x": _w((lambda *s: _rng.normal(s) * 0.05)(B, S, D)),
            "w1": _w((lambda *s: _rng.normal(s) * 0.05)(D, F)),
            "b1": _w((lambda *s: _rng.normal(s) * 0.05)(F)),
            "w2": _w((lambda *s: _rng.normal(s) * 0.05)(F, D)),
            "b2": _w((lambda *s: _rng.normal(s) * 0.05)(D)),
        }
    _B_in = _B_setup()

    return {
        "A_x": _A_in["x"],
        "A_wqkv": _A_in["wqkv"],
        "A_w_phi": _A_in["w_phi"],
        "A_wo": _A_in["wo"],
        "B_x": _B_in["x"],
        "B_w1": _B_in["w1"],
        "B_b1": _B_in["b1"],
        "B_w2": _B_in["w2"],
        "B_b2": _B_in["b2"],
    }

def reference(A_x, A_wqkv, A_w_phi, A_wo, B_x, B_w1, B_b1, B_w2, B_b2):
    def _A_ref(x, wqkv, w_phi, wo):
        B, S, D = x.shape
        H = 32; Dh = D // H
        qkv = (lambda x, *d: x.transpose(*d))((x @ wqkv).reshape(B, S, 3, H, Dh), 2, 0, 3, 1, 4)
        q, k, v = qkv[0], qkv[1], qkv[2]
        pq = jnp.einsum("bhsd,hdf->bhsf", q, w_phi)
        pk = jnp.einsum("bhsd,hdf->bhsf", k, w_phi)
        phi_q = jnp.concatenate([_softmax(pq, axis=-1), _softmax(-pq, axis=-1)], axis=-1)
        phi_k = jnp.concatenate([_softmax(pk, axis=-1), _softmax(-pk, axis=-1)], axis=-1)
        kv = jnp.einsum("bhsf,bhsd->bhfd", phi_k, v)
        z  = jnp.einsum("bhsf->bhf", phi_k)
        num = jnp.einsum("bhqf,bhfd->bhqd", phi_q, kv)
        den = jnp.einsum("bhqf,bhf->bhq", phi_q, z)[..., None] + 1e-6
        o = num / den
        return (lambda x, *d: x.transpose(*d))(o, 0, 2, 1, 3).reshape(B, S, D) @ wo

    def _B_ref(x, w1, b1, w2, b2):
        h = jnp.einsum("bsd,df->bsf", x, w1) + b1
        zero = jnp.zeros_like(h)
        r = jnp.where(h > zero, h, zero)
        h = r * r
        out = jnp.einsum("bsf,fd->bsd", h, w2) + b2
        return out

    x = A_x
    h = x + _A_ref(_layernorm(x, axis=-1), A_wqkv, A_w_phi, A_wo)
    h2 = h + _B_ref(_layernorm(h, axis=-1), B_w1, B_b1, B_w2, B_b2)
    return h2
```

```python
import functools
import numpy as np
import jax
import jax.numpy as jnp
from jax import lax
import jax.experimental.pallas as pl
import jax.experimental.pallas.tpu as pltpu

S, D, H, DH, F = 2048, 512, 32, 16, 1792
NG = 8
NTILE = S // 128
FH = F // 2
LOG2E = float(np.log2(np.e))
f32, bf16, u32 = jnp.float32, jnp.bfloat16, jnp.uint32
NT = (((1,), (1,)), ((), ()))


def _pk(x):
    return pltpu.bitcast(x.astype(bf16), u32)


def _up(x):
    return pltpu.bitcast(x, bf16)


def _ln(x):
    m = jnp.mean(x, axis=-1, keepdims=True)
    xc = x - m
    v = jnp.mean(xc * xc, axis=-1, keepdims=True)
    return xc * lax.rsqrt(v + 1e-5)


def _allred(op, x3):
    r = x3[0]
    for i in range(1, 8):
        r = op(r, x3[i])
    r = op(r, pltpu.roll(r, 4, axis=0))
    return r[None]


def _dual_exp(p):
    L = p.shape[1]
    p3 = p.reshape(8, 8, L)
    mx = _allred(jnp.maximum, p3)
    mn = _allred(jnp.minimum, p3)
    ep = jnp.exp2(p3 - mx)
    en = jnp.exp2(mn - p3)
    sp = _allred(jnp.add, ep)
    sn = _allred(jnp.add, en)
    return ep, en, sp, sn


def _rcp(x):
    r = pl.reciprocal(x, approx=True)
    return r * (2.0 - x * r)


def make_kernel(T=512, interpret=False, p2mode="swploop", wvt="xlu", flags=None, phiq=True, XC=(2, 2), ep=1, tb=13, npc=10, npc2=4):
    NB = S // T

    def kernel(x_hbm, wqkv_hbm, wphi_hbm, wo_hbm, w1_hbm, b1_hbm, w2_hbm, b2_hbm, out_hbm,
               x_v, xn_v, wq_v, wk_v, wv_v, wphi_v, wo_v, w1_v, w2_v, b1_v, b2_v,
               wqT_v, wkvT_v, phik_v, vT_v, z_v, kvt_v, phiq_v, h_v, out_v, w1s_v, w2s_v, sem_x, sem_w, sem_o):
        cp_phi = pltpu.make_async_copy(wphi_hbm, wphi_v, sem_w.at[0])
        cp_wk = pltpu.make_async_copy(wqkv_hbm.at[:, pl.ds(D, D)], wk_v, sem_w.at[1])
        cp_wv = pltpu.make_async_copy(wqkv_hbm.at[:, pl.ds(2 * D, D)], wv_v, sem_w.at[2])
        cp_wq = pltpu.make_async_copy(wqkv_hbm.at[:, pl.ds(0, D)], wq_v, sem_w.at[3])
        cp_wo = pltpu.make_async_copy(wo_hbm, wo_v, sem_w.at[4])
        cp_w1 = pltpu.make_async_copy(w1_hbm, w1_v, sem_w.at[5])
        cp_w2 = pltpu.make_async_copy(w2_hbm, w2_v, sem_w.at[6])
        cp_b1 = pltpu.make_async_copy(b1_hbm, b1_v, sem_w.at[7])
        cp_b2 = pltpu.make_async_copy(b2_hbm, b2_v, sem_w.at[8])
        n0, n1 = XC
        XCH = [(0, n0 * 128), (n0 * 128, n1 * 128), ((n0 + n1) * 128, S - (n0 + n1) * 128)]
        cp_x = [pltpu.make_async_copy(x_hbm.at[0, pl.ds(r0, n), :], x_v.at[pl.ds(r0, n), :], sem_x.at[i])
                for i, (r0, n) in enumerate(XCH)]
        cp_phi.start(); cp_x[0].start(); cp_wk.start(); cp_wv.start(); cp_x[1].start()

        def iota(shape, d):
            return lax.broadcasted_iota(jnp.int32, shape, d)
        m32 = iota((128, 32), 0)
        h32 = iota((128, 32), 1)
        hloc32 = (m32 // 64) * 4 + (m32 % 4)
        m256 = iota((128, 256), 0)
        c256 = iota((128, 256), 1)
        mask1 = ((m256 % 64) // 4) == (c256 % 16)
        sel = jnp.where((iota((256, 128), 0) // 16) == (iota((256, 128), 1) % 16), 1.0, 0.0).astype(bf16)
        m128 = iota((128, 128), 0)
        c128 = iota((128, 128), 1)
        mask2 = ((m128 // 64) * 4 + (m128 % 4)) == (c128 // 16)
        z_v[...] = jnp.zeros_like(z_v)
        cp_phi.wait()
        w2d = wphi_v[...].reshape(DH * DH, H)
        P = []
        for G in range(4):
            lg = jnp.where(h32 == hloc32 + G * 8, 1.0, 0.0).astype(bf16)
            rw = lax.dot_general(lg, w2d, NT, preferred_element_type=f32)
            rm = jnp.where(mask1, rw, 0.0).astype(bf16)
            q = jnp.dot(rm, sel, preferred_element_type=f32)
            P.append(jnp.where(mask2, q, 0.0).astype(bf16))

        def fold(w_ref, out_ref):
            for G in range(4):
                wt = lax.dot_general(P[G], w_ref[:, G * 128:(G + 1) * 128], NT, preferred_element_type=f32)
                out_ref[G * 64:(G + 1) * 64, :] = _pk(wt * LOG2E)
        cp_x[0].wait(); cp_wk.wait()
        cp_x[2].start()
        cp_w1.start(); cp_w2.start(); cp_b1.start(); cp_b2.start(); cp_wo.start(); cp_wq.start()
        fold(wk_v, wkvT_v)

        def ln1(t):
            xn_v[pl.ds(t * 64, 64), :] = _pk(_ln(x_v[pl.ds(t * 128, 128), :].astype(f32)))

        def xnb(t, n=1):
            return _up(xn_v[pl.ds(t * 64, n * 64), :])

        def sm_k(t, pkT):
            for g in range(NG):
                e_p, e_n, sp, sn = _dual_exp(pkT[g * 64:(g + 1) * 64, :])
                r = _rcp(sp * sn)
                php = (e_p * (r * sn)).reshape(64, 128)
                phn = (e_n * (r * sp)).reshape(64, 128)
                ph = jnp.concatenate([php, phn], axis=0)
                z_v[g * 128:(g + 1) * 128, :] += ph
                phik_v[g * 64:(g + 1) * 64, pl.ds(t * 128, 128)] = _pk(ph)

        def k_tile(t):
            sm_k(t, lax.dot_general(_up(wkvT_v[0:256, :]), xnb(t), NT, preferred_element_type=f32))

        def v_tile(t):
            vT_v[:, pl.ds(t * 128, 128)] = _pk(
                lax.dot_general(_up(wkvT_v[256:512, :]), xnb(t), NT, preferred_element_type=f32))

        def kv_tile(t):
            r = lax.dot_general(_up(wkvT_v[...]), xnb(t), NT, preferred_element_type=f32)
            vT_v[:, pl.ds(t * 128, 128)] = _pk(r[D:])
            sm_k(t, r[:D])

        def combo(w_ref, ws_ref, kh, nh, r0, c0, cw):
            b11 = w_ref[r0:r0 + RP, c0:c0 + cw].astype(f32)
            b12 = w_ref[r0:r0 + RP, nh + c0:nh + c0 + cw].astype(f32)
            b21 = w_ref[kh + r0:kh + r0 + RP, c0:c0 + cw].astype(f32)
            b22 = w_ref[kh + r0:kh + r0 + RP, nh + c0:nh + c0 + cw].astype(f32)
            ro = pl.ds(r0, RP)
            co = pl.ds(c0, cw)
            ws_ref[0, ro, co] = (b11 + b22).astype(bf16)
            ws_ref[1, ro, co] = (b12 - b22).astype(bf16)
            ws_ref[2, ro, co] = (b21 - b11).astype(bf16)
            ws_ref[3, ro, co] = (b11 + b12).astype(bf16)
            ws_ref[4, ro, co] = (b21 + b22).astype(bf16)

        RP = 32
        pieces = [(w1_v, w1s_v, 256, FH, r0, c0, min(256, FH - c0)) for r0 in range(0, 256, RP)
                  for c0 in range(0, FH, 256)]
        pieces += [(w2_v, w2s_v, FH, 256, r0, 0, 256) for r0 in range(0, FH, RP)]

        def do_pieces(n):
            for _ in range(min(n, len(pieces))):
                combo(*pieces.pop(0))

        def k_mm(t):
            return lax.dot_general(_up(wkvT_v[0:256, :]), xnb(t), NT, preferred_element_type=f32)

        for t in range(n0):
            ln1(t)
        for t in range(n0 - 2):
            k_tile(t)
        pk_held = k_mm(n0 - 2)
        cp_wv.wait(); cp_x[1].wait()
        pk_next = k_mm(n0 - 1)
        sm_k(n0 - 2, pk_held)
        if wvt == "xlu":
            wkvT_v[256:512, :] = _pk(jnp.transpose(wv_v[...].astype(f32)))
        else:
            eye = jnp.where(m128 == c128, 1.0, 0.0).astype(bf16)
            for G in range(4):
                wkvT_v[256 + G * 64:256 + (G + 1) * 64, :] = _pk(lax.dot_general(
                    eye, wv_v[:, G * 128:(G + 1) * 128], NT, preferred_element_type=f32))
        for t in range(n0, n0 + n1):
            ln1(t)
        sm_k(n0 - 1, pk_next)
        for t in range(n0, n0 + n1):
            k_tile(t)
        for t in range(n0 + n1 - 1):
            v_tile(t)
        cp_x[2].wait()
        v_tile(n0 + n1 - 1)
        for t in range(n0 + n1, NTILE):
            ln1(t)
        for t in range(n0 + n1, NTILE):
            if t == tb:
                cp_w1.wait(); cp_w2.wait(); cp_b1.wait(); cp_b2.wait(); cp_wo.wait(); cp_wq.wait()
            kv_tile(t)
            if t >= tb:
                do_pieces(npc)
        fold(wq_v, wqT_v)
        mk = iota((64, 128), 0)
        kk = iota((64, 128), 1)
        mask3 = (mk // 16) == (kk % 4)
        for g in range(NG):
            c = lax.dot_general(_up(vT_v[g * 32:(g + 1) * 32, :]), _up(phik_v[g * 64:(g + 1) * 64, :]), NT,
                                preferred_element_type=f32)
            kvt_v[g * 32:(g + 1) * 32, :] = _pk(jnp.where(mask3, c, 0.0))
            do_pieces(npc2)
        do_pieces(100)
        zsum = jnp.sum(z_v[...], axis=1, keepdims=True)
        z_v[...] = jnp.broadcast_to(zsum, z_v.shape)

        b1 = b1_v[...].astype(f32).reshape(1, F)
        b2 = b2_v[...].astype(f32).reshape(1, D)

        def q_tile(t0, j):
            pqT = lax.dot_general(_up(wqT_v[...]), _up(xn_v[pl.ds((t0 + j) * 64, 64), :]), NT,
                                  preferred_element_type=f32)
            out = []
            for g in range(NG):
                e_p, e_n, sp, sn = _dual_exp(pqT[g * 64:(g + 1) * 64, :])
                zp = z_v[g * 128:g * 128 + 64, :].reshape(8, 8, 128)
                zn = z_v[g * 128 + 64:(g + 1) * 128, :].reshape(8, 8, 128)
                w = _allred(jnp.add, e_p * zp) * sn + _allred(jnp.add, e_n * zn) * sp + 1e-6 * (sp * sn)
                r = _rcp(w)
                php = (e_p * (r * sn)).reshape(64, 128)
                phn = (e_n * (r * sp)).reshape(64, 128)
                ph = jnp.concatenate([php, phn], axis=0)
                if phiq:
                    phiq_v[g * 64:(g + 1) * 64, pl.ds(j * 128, 128)] = _pk(ph)
                else:
                    out.append(ph.astype(bf16))
            return out

        def q_blk(i):
            t0 = i * (T // 128)
            return [q_tile(t0, j) for j in range(T // 128)]

        def num(ph):
            os_ = []
            for j in range(T // 128):
                oT = []
                for g in range(NG):
                    rhs = _up(phiq_v[g * 64:(g + 1) * 64, pl.ds(j * 128, 128)]) if phiq else ph[j][g]
                    oT.append(jnp.dot(_up(kvt_v[g * 32:(g + 1) * 32, :]), rhs, preferred_element_type=f32))
                os_.append(jnp.transpose(jnp.concatenate(oT, axis=0)).astype(bf16))
            return jnp.concatenate(os_, axis=0)

        def resid(rows, o):
            return x_v[rows, :].astype(f32) + jnp.dot(o, wo_v[...], preferred_element_type=f32)

        def strassen(a11, a12, a21, a22, ws_ref, w):
            w_ref, kh, nh = w

            def mm(x, i):
                if i == 1:
                    rhs = w_ref[0:kh, 0:nh]
                elif i == 4:
                    rhs = w_ref[kh:2 * kh, nh:2 * nh]
                else:
                    rhs = ws_ref[{0: 0, 2: 1, 3: 2, 5: 3, 6: 4}[i]]
                return jnp.dot(x.astype(bf16), rhs, preferred_element_type=f32)
            m1 = mm(a11 + a22, 0)
            m2 = mm(a21 + a22, 1)
            m3 = mm(a11, 2)
            m4 = mm(a22, 3)
            m5 = mm(a11 + a12, 4)
            m6 = mm(a21 - a11, 5)
            m7 = mm(a12 - a22, 6)
            return m1 + m4 - m5 + m7, m3 + m5, m2 + m4, m1 - m2 + m3 + m6

        def ffn1(h):
            R = h.shape[0] // 2
            hn = _ln(h)
            c11, c12, c21, c22 = strassen(hn[:R, :256], hn[:R, 256:], hn[R:, :256], hn[R:, 256:], w1s_v,
                                          (w1_v, 256, FH))

            def act(c, b):
                r = jnp.maximum(c + b, 0.0)
                return r * r
            bl, br = b1[:, :FH], b1[:, FH:]
            return act(c11, bl), act(c12, br), act(c21, bl), act(c22, br)

        def ffn2(rows, h, a, sem):
            R = h.shape[0] // 2
            o11, o12, o21, o22 = strassen(*a, w2s_v, (w2_v, FH, 256))
            top, bot = rows
            out_v[top, 0:256] = (h[:R, :256] + (o11 + b2[:, :256])).astype(bf16)
            out_v[top, 256:512] = (h[:R, 256:] + (o12 + b2[:, 256:])).astype(bf16)
            out_v[bot, 0:256] = (h[R:, :256] + (o21 + b2[:, :256])).astype(bf16)
            out_v[bot, 256:512] = (h[R:, 256:] + (o22 + b2[:, 256:])).astype(bf16)
            pltpu.make_async_copy(out_v.at[top, :], out_hbm.at[0, top, :], sem.at[0]).start()
            pltpu.make_async_copy(out_v.at[bot, :], out_hbm.at[0, bot, :], sem.at[1]).start()

        def blk(i, n=T, off=0):
            if isinstance(i, int):
                return pl.ds(i * T + off, n)
            return pl.ds(pl.multiple_of(i * T + off, 128), n)

        if p2mode in ("swp", "swploop"):
            o = num(q_blk(0))
            h_v[...] = resid(blk(0), o)

            def body(i, carry):
                ph = q_blk(i + 1)
                h = h_v[...]
                a = ffn1(h)
                o = num(ph)
                ffn2((blk(i, T // 2), blk(i, T // 2, T // 2)), h, a, sem_o.at[i])
                h_v[...] = resid(blk(i + 1), o)
                return carry
            if p2mode == "swp":
                for i in range(NB - 1):
                    body(i, 0)
            else:
                lax.fori_loop(0, NB - 1, body, 0)
            Te = T // ep
            hs = [h_v[pl.ds(e * Te, Te), :] for e in range(ep)]
            As = [ffn1(hs[e]) for e in range(ep)]
            for e in range(ep):
                ffn2((blk(NB - 1, Te // 2, e * Te), blk(NB - 1, Te // 2, e * Te + Te // 2)), hs[e], As[e],
                     sem_o.at[NB - 1 + e])
        for i in range(NB - 1):
            for u in range(2):
                rows = blk(i, T // 2, u * (T // 2))
                pltpu.make_async_copy(out_v.at[rows, :], out_hbm.at[0, rows, :], sem_o.at[i, u]).wait()
        for e in range(ep):
            for u in range(2):
                rows = blk(NB - 1, T // ep // 2, e * (T // ep) + u * (T // ep // 2))
                pltpu.make_async_copy(out_v.at[rows, :], out_hbm.at[0, rows, :], sem_o.at[NB - 1 + e, u]).wait()

    any_spec = pl.BlockSpec(memory_space=pl.ANY)
    scratch = [
        pltpu.VMEM((S, D), bf16), pltpu.VMEM((S // 2, D), u32),
        pltpu.VMEM((D, D), bf16), pltpu.VMEM((D, D), bf16), pltpu.VMEM((D, D), bf16),
        pltpu.VMEM((DH, DH, H), bf16), pltpu.VMEM((D, D), bf16),
        pltpu.VMEM((D, F), bf16), pltpu.VMEM((F, D), bf16),
        pltpu.VMEM((F,), bf16), pltpu.VMEM((D,), bf16),
        pltpu.VMEM((D // 2, D), u32), pltpu.VMEM((D, D), u32),
        pltpu.VMEM((D, S), u32), pltpu.VMEM((D // 2, S), u32), pltpu.VMEM((2 * D, 128), f32),
        pltpu.VMEM((D // 2, 128), u32), pltpu.VMEM((D, T), u32), pltpu.VMEM((T, D), f32), pltpu.VMEM((S, D), bf16),
        pltpu.VMEM((5, 256, FH), bf16), pltpu.VMEM((5, FH, 256), bf16),
        pltpu.SemaphoreType.DMA((3,)), pltpu.SemaphoreType.DMA((9,)), pltpu.SemaphoreType.DMA((NB + 3, 2)),
    ]

    @jax.jit
    def run(A_x, A_wqkv, A_w_phi, A_wo, B_x, B_w1, B_b1, B_w2, B_b2):
        return pl.pallas_call(
            kernel,
            out_shape=jax.ShapeDtypeStruct((1, S, D), bf16),
            in_specs=[any_spec] * 8,
            out_specs=any_spec,
            scratch_shapes=scratch,
            compiler_params=pltpu.CompilerParams(vmem_limit_bytes=100 * 1024 * 1024, flags=flags),
            interpret=interpret,
            name="mytest",
        )(A_x, A_wqkv, jnp.transpose(A_w_phi, (1, 2, 0)), A_wo, B_w1, B_b1, B_w2, B_b2)
    return run


_run = make_kernel(ep=4)


@jax.jit
def pallas_sequential_preLN__linear_kernel_hedgehog__dense_activation_squared_relu__prompt_kernel(
    A_x: jax.Array,
    A_wqkv: jax.Array,
    A_w_phi: jax.Array,
    A_wo: jax.Array,
    B_x: jax.Array,
    B_w1: jax.Array,
    B_b1: jax.Array,
    B_w2: jax.Array,
    B_b2: jax.Array,
):
    return _run(A_x, A_wqkv, A_w_phi, A_wo, B_x, B_w1, B_b1, B_w2, B_b2)
```

```python
import functools
import numpy as np
import jax
import jax.numpy as jnp
from jax import lax
import jax.experimental.pallas as pl
import jax.experimental.pallas.tpu as pltpu

S, D, H, DH, F = 2048, 512, 32, 16, 1792
NG = 8
NTILE = S // 128
FH = F // 2
LOG2E = float(np.log2(np.e))
f32, bf16, u32 = jnp.float32, jnp.bfloat16, jnp.uint32
NT = (((1,), (1,)), ((), ()))


def _pk(x):
    return pltpu.bitcast(x.astype(bf16), u32)


def _up(x):
    return pltpu.bitcast(x, bf16)


def _ln(x):
    m = jnp.mean(x, axis=-1, keepdims=True)
    xc = x - m
    v = jnp.mean(xc * xc, axis=-1, keepdims=True)
    return xc * lax.rsqrt(v + 1e-5)


def _allred(op, x3):
    r = x3[0]
    for i in range(1, 8):
        r = op(r, x3[i])
    r = op(r, pltpu.roll(r, 4, axis=0))
    return r[None]


def _dual_exp(p):
    L = p.shape[1]
    p3 = p.reshape(8, 8, L)
    mx = _allred(jnp.maximum, p3)
    mn = _allred(jnp.minimum, p3)
    ep = jnp.exp2(p3 - mx)
    en = jnp.exp2(mn - p3)
    sp = _allred(jnp.add, ep)
    sn = _allred(jnp.add, en)
    return ep, en, sp, sn


def _rcp(x):
    r = pl.reciprocal(x, approx=True)
    return r * (2.0 - x * r)


def make_kernel(T=512, interpret=False, p2mode="swploop", wvt="xlu", flags=None, phiq=True, XC=(2, 2), ep=1, tb=13, npc=64, npc2=10, usedep=True, rp=8, swo=True, kmid=6, nl=None, epi=True, dend=True, eps=True):
    NB = S // T
    Te = T // ep
    nl = NB - 1 if nl is None else nl

    def kernel(x_hbm, wqkv_hbm, wphi_hbm, wo_hbm, w1_hbm, b1_hbm, w2_hbm, b2_hbm, out_hbm,
               x_v, xn_v, wq_v, wk_v, wv_v, wphi_v, wo_v, w1_v, w2_v, b1_v, b2_v,
               wqT_v, wkvT_v, phik_v, vT_v, z_v, kvt_v, phiq_v, h_v, out_v, w1s_v, w2s_v, hA_v, wos_v, sem_x, sem_w, sem_o):
        cp_phi = pltpu.make_async_copy(wphi_hbm, wphi_v, sem_w.at[0])
        cp_wk = pltpu.make_async_copy(wqkv_hbm.at[:, pl.ds(D, D)], wk_v, sem_w.at[1])
        cp_wv = pltpu.make_async_copy(wqkv_hbm.at[:, pl.ds(2 * D, D)], wv_v, sem_w.at[2])
        cp_wq = pltpu.make_async_copy(wqkv_hbm.at[:, pl.ds(0, D)], wq_v, sem_w.at[3])
        cp_wo = pltpu.make_async_copy(wo_hbm, wo_v, sem_w.at[4])
        cp_w1 = pltpu.make_async_copy(w1_hbm, w1_v, sem_w.at[5])
        cp_w2 = pltpu.make_async_copy(w2_hbm, w2_v, sem_w.at[6])
        cp_b1 = pltpu.make_async_copy(b1_hbm, b1_v, sem_w.at[7])
        cp_b2 = pltpu.make_async_copy(b2_hbm, b2_v, sem_w.at[8])
        n0, n1 = XC
        XCH = [(0, n0 * 128), (n0 * 128, n1 * 128), ((n0 + n1) * 128, S - (n0 + n1) * 128)]
        cp_x = [pltpu.make_async_copy(x_hbm.at[0, pl.ds(r0, n), :], x_v.at[pl.ds(r0, n), :], sem_x.at[i])
                for i, (r0, n) in enumerate(XCH)]
        cp_phi.start(); cp_x[0].start(); cp_wk.start(); cp_wv.start(); cp_x[1].start()

        def iota(shape, d):
            return lax.broadcasted_iota(jnp.int32, shape, d)
        m32 = iota((128, 32), 0)
        h32 = iota((128, 32), 1)
        hloc32 = (m32 // 64) * 4 + (m32 % 4)
        m256 = iota((128, 256), 0)
        c256 = iota((128, 256), 1)
        mask1 = ((m256 % 64) // 4) == (c256 % 16)
        sel = jnp.where((iota((256, 128), 0) // 16) == (iota((256, 128), 1) % 16), 1.0, 0.0).astype(bf16)
        m128 = iota((128, 128), 0)
        c128 = iota((128, 128), 1)
        mask2 = ((m128 // 64) * 4 + (m128 % 4)) == (c128 // 16)
        z_v[...] = jnp.zeros_like(z_v)
        cp_phi.wait()
        w2d = wphi_v[...].reshape(DH * DH, H)
        P = []
        for G in range(4):
            lg = jnp.where(h32 == hloc32 + G * 8, 1.0, 0.0).astype(bf16)
            rw = lax.dot_general(lg, w2d, NT, preferred_element_type=f32)
            rm = jnp.where(mask1, rw, 0.0).astype(bf16)
            q = jnp.dot(rm, sel, preferred_element_type=f32)
            P.append(jnp.where(mask2, q, 0.0).astype(bf16))

        def fold(w_ref, out_ref):
            for G in range(4):
                wt = lax.dot_general(P[G], w_ref[:, G * 128:(G + 1) * 128], NT, preferred_element_type=f32)
                out_ref[G * 64:(G + 1) * 64, :] = _pk(wt * LOG2E)
        cp_x[0].wait(); cp_wk.wait()
        cp_x[2].start()
        cp_w1.start(); cp_w2.start(); cp_b1.start(); cp_b2.start(); cp_wo.start(); cp_wq.start()
        fold(wk_v, wkvT_v)

        def ln1(t):
            xn_v[pl.ds(t * 64, 64), :] = _pk(_ln(x_v[pl.ds(t * 128, 128), :].astype(f32)))

        def xnb(t, n=1):
            return _up(xn_v[pl.ds(t * 64, n * 64), :])

        def sm_k(t, pkT):
            for g in range(NG):
                e_p, e_n, sp, sn = _dual_exp(pkT[g * 64:(g + 1) * 64, :])
                r = _rcp(sp * sn)
                php = (e_p * (r * sn)).reshape(64, 128)
                phn = (e_n * (r * sp)).reshape(64, 128)
                ph = jnp.concatenate([php, phn], axis=0)
                z_v[g * 128:(g + 1) * 128, :] += ph
                phik_v[g * 64:(g + 1) * 64, pl.ds(t * 128, 128)] = _pk(ph)

        def k_tile(t):
            sm_k(t, lax.dot_general(_up(wkvT_v[0:256, :]), xnb(t), NT, preferred_element_type=f32))

        def v_tile(t):
            vT_v[:, pl.ds(t * 128, 128)] = _pk(
                lax.dot_general(_up(wkvT_v[256:512, :]), xnb(t), NT, preferred_element_type=f32))

        def kv_tile(t):
            r = lax.dot_general(_up(wkvT_v[...]), xnb(t), NT, preferred_element_type=f32)
            vT_v[:, pl.ds(t * 128, 128)] = _pk(r[D:])
            sm_k(t, r[:D])
            return r

        def combo(w_ref, ws_ref, kh, nh, r0, c0, cw, dep):
            b11 = w_ref[r0:r0 + RP, c0:c0 + cw].astype(f32)
            b12 = w_ref[r0:r0 + RP, nh + c0:nh + c0 + cw].astype(f32)
            b21 = w_ref[kh + r0:kh + r0 + RP, c0:c0 + cw].astype(f32)
            b22 = w_ref[kh + r0:kh + r0 + RP, nh + c0:nh + c0 + cw].astype(f32)
            if dep is not None:
                z = jnp.concatenate([jnp.concatenate([dep] * (RP // 8), axis=0)] * (cw // 128), axis=1)
                b11 = pltpu.bitcast(pltpu.bitcast(b11, u32) | z, f32)
                b22 = pltpu.bitcast(pltpu.bitcast(b22, u32) | z, f32)
            ro = pl.ds(r0, RP)
            co = pl.ds(c0, cw)
            ws_ref[0, ro, co] = (b11 + b22).astype(bf16)
            ws_ref[1, ro, co] = (b12 - b22).astype(bf16)
            ws_ref[2, ro, co] = (b21 - b11).astype(bf16)
            ws_ref[3, ro, co] = (b11 + b12).astype(bf16)
            ws_ref[4, ro, co] = (b21 + b22).astype(bf16)

        RP = rp
        pieces = [(w1_v, w1s_v, 256, FH, r0, c0, min(256, FH - c0)) for r0 in range(0, 256, RP)
                  for c0 in range(0, FH, 256)]
        pieces += [(w2_v, w2s_v, FH, 256, r0, 0, 256) for r0 in range(0, FH, RP)]
        if swo:
            pieces = [(wo_v, wos_v, 256, 256, r0, 0, 256) for r0 in range(0, 256, RP)] + pieces

        def do_pieces(n, r=None):
            n = min(n, len(pieces))
            for j in range(n):
                dep = None
                if r is not None and usedep:
                    r0 = 8 * ((j * (r.shape[0] // 8)) // n)
                    dep = (pltpu.bitcast(r[r0:r0 + 8, 0:128], u32) & 1) >> 1
                combo(*pieces.pop(0), dep)

        def k_mm(t):
            return lax.dot_general(_up(wkvT_v[0:256, :]), xnb(t), NT, preferred_element_type=f32)

        for t in range(n0):
            ln1(t)
        for t in range(n0 - 2):
            k_tile(t)
        pk_held = k_mm(n0 - 2)
        cp_wv.wait(); cp_x[1].wait()
        pk_next = k_mm(n0 - 1)
        sm_k(n0 - 2, pk_held)
        if wvt == "xlu":
            wkvT_v[256:512, :] = _pk(jnp.transpose(wv_v[...].astype(f32)))
        else:
            eye = jnp.where(m128 == c128, 1.0, 0.0).astype(bf16)
            for G in range(4):
                wkvT_v[256 + G * 64:256 + (G + 1) * 64, :] = _pk(lax.dot_general(
                    eye, wv_v[:, G * 128:(G + 1) * 128], NT, preferred_element_type=f32))
        for t in range(n0, n0 + n1):
            ln1(t)
        sm_k(n0 - 1, pk_next)
        for t in range(n0, n0 + n1):
            k_tile(t)
        for t in range(n0 + n1 - 1):
            v_tile(t)
        cp_x[2].wait()
        v_tile(n0 + n1 - 1)
        for t in range(n0 + n1, NTILE):
            ln1(t)
        for t in range(n0 + n1, NTILE):
            if t == tb:
                cp_w1.wait(); cp_w2.wait(); cp_b1.wait(); cp_b2.wait(); cp_wo.wait(); cp_wq.wait()
            r = kv_tile(t)
            if t >= tb:
                do_pieces(npc, r)
        fold(wq_v, wqT_v)
        mk = iota((64, 128), 0)
        kk = iota((64, 128), 1)
        mask3 = (mk // 16) == (kk % 4)
        for g in range(NG):
            c = lax.dot_general(_up(vT_v[g * 32:(g + 1) * 32, :]), _up(phik_v[g * 64:(g + 1) * 64, :]), NT,
                                preferred_element_type=f32)
            kvt_v[g * 32:(g + 1) * 32, :] = _pk(jnp.where(mask3, c, 0.0))
            do_pieces(npc2, c)
        do_pieces(10 ** 6)
        zsum = jnp.sum(z_v[...], axis=1, keepdims=True)
        z_v[...] = jnp.broadcast_to(zsum, z_v.shape)

        b1 = b1_v[...].astype(f32).reshape(1, F)
        b2 = b2_v[...].astype(f32).reshape(1, D)

        def q_tile(t0, j):
            pqT = lax.dot_general(_up(wqT_v[...]), _up(xn_v[pl.ds((t0 + j) * 64, 64), :]), NT,
                                  preferred_element_type=f32)
            out = []
            for g in range(NG):
                e_p, e_n, sp, sn = _dual_exp(pqT[g * 64:(g + 1) * 64, :])
                zp = z_v[g * 128:g * 128 + 64, :].reshape(8, 8, 128)
                zn = z_v[g * 128 + 64:(g + 1) * 128, :].reshape(8, 8, 128)
                w = _allred(jnp.add, e_p * zp) * sn + _allred(jnp.add, e_n * zn) * sp + 1e-6 * (sp * sn)
                r = _rcp(w)
                php = (e_p * (r * sn)).reshape(64, 128)
                phn = (e_n * (r * sp)).reshape(64, 128)
                ph = jnp.concatenate([php, phn], axis=0)
                if phiq:
                    phiq_v[g * 64:(g + 1) * 64, pl.ds(j * 128, 128)] = _pk(ph)
                else:
                    out.append(ph.astype(bf16))
            return out

        def q_blk(i):
            t0 = i * (T // 128)
            return [q_tile(t0, j) for j in range(T // 128)]

        def num(ph, e):
            os_ = []
            for j in range(e * Te // 128, (e + 1) * Te // 128):
                oT = []
                for g in range(NG):
                    rhs = _up(phiq_v[g * 64:(g + 1) * 64, pl.ds(j * 128, 128)]) if phiq else ph[j][g]
                    oT.append(jnp.dot(_up(kvt_v[g * 32:(g + 1) * 32, :]), rhs, preferred_element_type=f32))
                os_.append(jnp.transpose(jnp.concatenate(oT, axis=0)))
            return jnp.concatenate(os_, axis=0)

        def resid(rows, o):
            return x_v[rows, :].astype(f32) + jnp.dot(o, wo_v[...], preferred_element_type=f32)

        def a_ops(a11, a12, a21, a22):
            return [a11 + a22, a21 + a22, a11, a22, a11 + a12, a21 - a11, a12 - a22]

        def strassen(ops, ws_ref, w, mid=None):
            w_ref, kh, nh = w
            ms = []
            for i in range(7):
                if mid is not None and i == kmid:
                    mid()
                if i == 1:
                    rhs = w_ref[0:kh, 0:nh]
                elif i == 4:
                    rhs = w_ref[kh:2 * kh, nh:2 * nh]
                else:
                    rhs = ws_ref[{0: 0, 2: 1, 3: 2, 5: 3, 6: 4}[i]]
                ms.append(jnp.dot(ops[i], rhs, preferred_element_type=f32))
            m1, m2, m3, m4, m5, m6, m7 = ms
            return m1 + m4 - m5 + m7, m3 + m5, m2 + m4, m1 - m2 + m3 + m6

        def ln2(h, e):
            hn = _ln(h)
            R = Te // 2
            ops = a_ops(hn[:R, :256], hn[:R, 256:], hn[R:, :256], hn[R:, 256:])
            for k in range(7):
                hA_v[k, pl.ds(e * (R // 2), R // 2), :] = _pk(ops[k])

        def ffn1(e0=0, ne=None, mid=None):
            ne = ep if ne is None else ne
            R2 = Te // 4
            ops = [_up(hA_v[k, pl.ds(e0 * R2, ne * R2), :]) for k in range(7)]
            c11, c12, c21, c22 = strassen(ops, w1s_v, (w1_v, 256, FH), mid)

            def act(c, b):
                r = jnp.maximum(c + b, 0.0)
                return r * r
            bl, br = b1[:, :FH], b1[:, FH:]
            return act(c11, bl), act(c12, br), act(c21, bl), act(c22, br)

        def ffn2(i, a, e0=0, ne=None):
            ne = ep if ne is None else ne
            ops = [x.astype(bf16) for x in a_ops(*a)]
            o11, o12, o21, o22 = strassen(ops, w2s_v, (w2_v, FH, 256))
            R = Te // 2
            for e in range(ne):
                top = blk(i, R, (e0 + e) * Te)
                bot = blk(i, R, (e0 + e) * Te + R)
                sl = slice(e * R, (e + 1) * R)
                out_v[top, 0:256] = (h_v[top, 0:256] + (o11[sl] + b2[:, :256])).astype(bf16)
                out_v[top, 256:512] = (h_v[top, 256:512] + (o12[sl] + b2[:, 256:])).astype(bf16)
                out_v[bot, 0:256] = (h_v[bot, 0:256] + (o21[sl] + b2[:, :256])).astype(bf16)
                out_v[bot, 256:512] = (h_v[bot, 256:512] + (o22[sl] + b2[:, 256:])).astype(bf16)
                if not dend:
                    both = blk(i, Te, (e0 + e) * Te)
                    pltpu.make_async_copy(out_v.at[both, :], out_hbm.at[0, both, :], sem_o.at[i, e0 + e]).start()
            if dend:
                for e in range(ne):
                    both = blk(i, Te, (e0 + e) * Te)
                    pltpu.make_async_copy(out_v.at[both, :], out_hbm.at[0, both, :], sem_o.at[i, e0 + e]).start()

        def blk(i, n=T, off=0):
            if isinstance(i, int):
                return pl.ds(i * T + off, n)
            return pl.ds(pl.multiple_of(i * T + off, 128), n)

        def attn_out(i, os_):
            for e in range(ep):
                rows = blk(i, Te, e * Te)
                o = os_[e]
                if swo:
                    R = Te // 2
                    ops = [x.astype(bf16) for x in a_ops(o[:R, :256], o[:R, 256:], o[R:, :256], o[R:, 256:])]
                    c11, c12, c21, c22 = strassen(ops, wos_v, (wo_v, 256, 256))
                    r = jnp.concatenate([jnp.concatenate([c11, c12], axis=1), jnp.concatenate([c21, c22], axis=1)], axis=0)
                else:
                    r = jnp.dot(o.astype(bf16), wo_v[...], preferred_element_type=f32)
                h = x_v[rows, :].astype(f32) + r
                h_v[rows, :] = h
                ln2(h, e)

        ph0 = q_blk(0)
        attn_out(0, [num(ph0, e) for e in range(ep)])

        def body(i, carry):
            ph = q_blk(i + 1)
            os_ = []
            a = ffn1(mid=lambda: os_.extend(num(ph, e) for e in range(ep)))
            attn_out(i + 1, os_)
            ffn2(i, a)
            return carry
        if p2mode == "swp":
            for i in range(NB - 1):
                body(i, 0)
        else:
            lax.fori_loop(0, nl, body, 0)
        if not epi:
            pass
        elif eps:
            As = [ffn1(e, 1) for e in range(ep)]
            for e in range(ep):
                ffn2(NB - 1, As[e], e, 1)
        else:
            ffn2(NB - 1, ffn1())
        for i in list(range(nl)) + ([NB - 1] if epi else []):
            for e in range(ep):
                rows = blk(i, Te, e * Te)
                pltpu.make_async_copy(out_v.at[rows, :], out_hbm.at[0, rows, :], sem_o.at[i, e]).wait()

    any_spec = pl.BlockSpec(memory_space=pl.ANY)
    scratch = [
        pltpu.VMEM((S, D), bf16), pltpu.VMEM((S // 2, D), u32),
        pltpu.VMEM((D, D), bf16), pltpu.VMEM((D, D), bf16), pltpu.VMEM((D, D), bf16),
        pltpu.VMEM((DH, DH, H), bf16), pltpu.VMEM((D, D), bf16),
        pltpu.VMEM((D, F), bf16), pltpu.VMEM((F, D), bf16),
        pltpu.VMEM((F,), bf16), pltpu.VMEM((D,), bf16),
        pltpu.VMEM((D // 2, D), u32), pltpu.VMEM((D, D), u32),
        pltpu.VMEM((D, S), u32), pltpu.VMEM((D // 2, S), u32), pltpu.VMEM((2 * D, 128), f32),
        pltpu.VMEM((D // 2, 128), u32), pltpu.VMEM((D, T), u32), pltpu.VMEM((S, D), f32), pltpu.VMEM((S, D), bf16),
        pltpu.VMEM((5, 256, FH), bf16), pltpu.VMEM((5, FH, 256), bf16),
        pltpu.VMEM((7, T // 4, 256), u32), pltpu.VMEM((5, 256, 256), bf16),
        pltpu.SemaphoreType.DMA((3,)), pltpu.SemaphoreType.DMA((9,)), pltpu.SemaphoreType.DMA((NB, ep)),
    ]

    @jax.jit
    def run(A_x, A_wqkv, A_w_phi, A_wo, B_x, B_w1, B_b1, B_w2, B_b2):
        return pl.pallas_call(
            kernel,
            out_shape=jax.ShapeDtypeStruct((1, S, D), bf16),
            in_specs=[any_spec] * 8,
            out_specs=any_spec,
            scratch_shapes=scratch,
            compiler_params=pltpu.CompilerParams(vmem_limit_bytes=100 * 1024 * 1024, flags=flags),
            interpret=interpret,
            name="hedgehog_block",
        )(A_x, A_wqkv, jnp.transpose(A_w_phi, (1, 2, 0)), A_wo, B_w1, B_b1, B_w2, B_b2)
    return run


_run = make_kernel(ep=2)


@jax.jit
def pallas_sequential_preLN__linear_kernel_hedgehog__dense_activation_squared_relu__prompt_kernel(
    A_x: jax.Array,
    A_wqkv: jax.Array,
    A_w_phi: jax.Array,
    A_wo: jax.Array,
    B_x: jax.Array,
    B_w1: jax.Array,
    B_b1: jax.Array,
    B_w2: jax.Array,
    B_b2: jax.Array,
):
    return _run(A_x, A_wqkv, A_w_phi, A_wo, B_x, B_w1, B_b1, B_w2, B_b2)
```
